```python
import jax
import jax.numpy as jnp

def _softmax(x, axis=-1):
    return jax.nn.softmax(x, axis=axis)
def _gelu(x):
    return jax.nn.gelu(x, approximate=True)
def _silu(x):
    return jax.nn.silu(x)
def _sigmoid(x):
    return jax.nn.sigmoid(x)
def _layernorm(x, axis=-1, eps=1e-5):
    m = jnp.mean(x, axis=axis, keepdims=True)
    v = jnp.var(x, axis=axis, keepdims=True)
    return (x - m) / jnp.sqrt(v + eps)
def _scatter_add(tgt, idx, src, axis=0):
    return tgt.at[idx].add(src)
def _segment_sum(src, seg, n):
    return jax.ops.segment_sum(src, seg, n)
class _Rng:
    def __init__(self, key):
        self._k = key
    def _next(self):
        self._k, sub = jax.random.split(self._k)
        return sub
    def normal(self, shape):
        return jax.random.normal(self._next(), shape, dtype=jnp.bfloat16)
    def randint(self, lo, hi, shape):
        return jax.random.randint(self._next(), shape, lo, hi, dtype=jnp.int32)
    def uniform(self, shape, lo=0.0, hi=1.0):
        return jax.random.uniform(self._next(), shape, jnp.bfloat16, lo, hi)
    def permutation(self, n):
        return jax.random.permutation(self._next(), n)


kernel_name = 'standalone__winograd__vision'

def setup_inputs():
    _rng = _Rng(jax.random.key(int.from_bytes(__import__("os").urandom(4), "little")))
    _w = (lambda a: (lambda t: t.astype(jnp.bfloat16) if jnp.issubdtype(t.dtype, jnp.floating) else t)(jnp.asarray(a)))
    H = W = 512 // 2 * 2
    C = 192
    return {
        "x": _w((lambda *s: _rng.normal(s) * 0.05)(1, H, W, C)),
        "w": _w((lambda *s: _rng.normal(s) * 0.05)(3, 3, C, C)),
    }

def reference(x, w):
    N, H, W, C = x.shape
    K = w.shape[-1]
    G  = jnp.array([[1.0,0.0,0.0],[0.5,0.5,0.5],[0.5,-0.5,0.5],[0.0,0.0,1.0]], dtype=x.dtype)
    Bt = jnp.array([[1.0,0.0,-1.0,0.0],[0.0,1.0,1.0,0.0],[0.0,-1.0,1.0,0.0],[0.0,1.0,0.0,-1.0]], dtype=x.dtype)
    At = jnp.array([[1.0,1.0,1.0,0.0],[0.0,1.0,-1.0,-1.0]], dtype=x.dtype)
    U = jnp.einsum("ar,rsck,bs->abck", G, w, G)
    xp = jnp.pad(x, ((0,0),(1,1),(1,1),(0,0)))
    nH, nW = H // 2, W // 2
    patches = []
    for i in range(4):
        for j in range(4):
            patches.append(xp[:, i:i + 2 * nH:2, j:j + 2 * nW:2, :])
    d = jnp.stack(patches).reshape(4, 4, N * nH * nW, C)
    V = jnp.einsum("ai,ijpc,bj->abpc", Bt, d, Bt)
    M = jnp.einsum("abck,abpc->abpk", U, V)
    Y = jnp.einsum("ma,abpk,nb->pmnk", At, M, At)
    Y = Y.reshape(N, nH, nW, 2, 2, K)
    Y = (lambda x, *d: x.transpose(*d))(Y, 0, 1, 3, 2, 4, 5).reshape(N, H, W, K)
    return Y
```

```python
import functools
from fractions import Fraction

import numpy as np
import jax
import jax.numpy as jnp
import jax.experimental.pallas as pl
import jax.experimental.pallas.tpu as pltpu


M_TILE = 6
_PTS = {2: [0, 1, -1], 4: [0, 1, -1, 2, -2],
        6: [0, 1, -1, 2, -2, Fraction(1, 2), Fraction(-1, 2)]}


def _polymul(a, b):
    out = [Fraction(0)] * (len(a) + len(b) - 1)
    for i, x in enumerate(a):
        for j, y in enumerate(b):
            out[i + j] += x * y
    return out


def _wino(m, pts):
    n = m + 2
    pts = [Fraction(p) for p in pts]
    at = [[pts[j] ** i if j < n - 1 else Fraction(int(i == m - 1))
           for j in range(n)] for i in range(m)]
    g, bt = [], []
    for i in range(n - 1):
        den = Fraction(1)
        q = [Fraction(1)]
        for k in range(n - 1):
            if k != i:
                den *= pts[i] - pts[k]
                q = _polymul(q, [-pts[k], Fraction(1)])
        g.append([pts[i] ** j / den for j in range(3)])
        bt.append(q + [Fraction(0)] * (n - len(q)))
    g.append([Fraction(0), Fraction(0), Fraction(1)])
    q = [Fraction(1)]
    for p in pts:
        q = _polymul(q, [-p, Fraction(1)])
    bt.append(q)
    return at, g, bt


def _lin(coefs, vals):
    acc = None
    terms = sorted([(c, v) for c, v in zip(coefs, vals) if c != 0],
                   key=lambda t: 0 if t[0] == 1 else 1)
    for c, v in terms:
        if acc is None:
            acc = v if c == 1 else v * float(c)
        elif c == 1:
            acc = acc + v
        elif c == -1:
            acc = acc - v
        else:
            acc = acc + v * float(c)
    return acc


def _in_tf(bt, d):
    n = len(d)
    out = [None] * n
    out[0] = _lin(bt[0], d)
    out[n - 1] = _lin(bt[n - 1], d)
    for a in range(1, n - 1, 2):
        ev = [c if j % 2 == 0 else 0 for j, c in enumerate(bt[a])]
        od = [c if j % 2 == 1 else 0 for j, c in enumerate(bt[a])]
        assert all(bt[a + 1][j] == (-od[j] if j % 2 else ev[j]) for j in range(n)) or \
            all(bt[a + 1][j] == (od[j] if j % 2 else -ev[j]) for j in range(n))
        e, o = _lin(ev, d), _lin(od, d)
        out[a] = e + o
        if all(bt[a + 1][j] == (-od[j] if j % 2 else ev[j]) for j in range(n)):
            out[a + 1] = e - o
        else:
            out[a + 1] = o - e
    return out


def _out_tf(at, mm):
    n = len(mm)
    s = [mm[a] + mm[a + 1] for a in range(1, n - 1, 2)]
    df = [mm[a] - mm[a + 1] for a in range(1, n - 1, 2)]
    ys = []
    for i, row in enumerate(at):
        src = s if i % 2 == 0 else df
        coefs = [row[a] for a in range(1, n - 1, 2)] + [row[0], row[n - 1]]
        ys.append(_lin(coefs, src + [mm[0], mm[n - 1]]))
    return ys


def _kernel(x_hbm, w_ref, o_hbm, xbuf, ut, v0, v1, m0, m1, ob0, ob1, isem, osem,
            *, H, C, W, m):
    n = m + 2
    at, g, bt = _wino(m, _PTS[m])
    nt = -(-H // m)
    nin_last = H - (m * (nt - 1) + 1)
    nout_last = H - m * (nt - 1)
    NS = 4
    nj = W // 128
    nc = C // 16
    vb, mb, ob = (v0, v1), (m0, m1), (ob0, ob1)
    f32, bf16 = jnp.float32, jnp.bfloat16

    def in_copy(c, rows):
        slot = c % NS
        return pltpu.make_async_copy(
            x_hbm.at[pl.ds(m * c + 1, rows)], xbuf.at[slot, pl.ds(0, rows)], isem.at[slot])

    def in_start(c):
        if c < nt - 1:
            in_copy(c, m).start()
        elif c == nt - 1:
            if nin_last > 0:
                in_copy(c, nin_last).start()
            xbuf[c % NS, nin_last:] = jnp.zeros((m - nin_last, C, W), bf16)

    def in_wait(c):
        if c < nt - 1:
            in_copy(c, m).wait()
        elif c == nt - 1 and nin_last > 0:
            in_copy(c, nin_last).wait()

    def out_copy(t, p, rows):
        return pltpu.make_async_copy(
            ob[p].at[pl.ds(0, rows)], o_hbm.at[pl.ds(m * t, rows)], osem.at[p])

    first = pltpu.make_async_copy(
        x_hbm.at[pl.ds(0, 1)], xbuf.at[NS - 1, pl.ds(m - 1, 1)], isem.at[NS - 1])
    first.start()
    for c in range(3):
        in_start(c)
    xbuf[NS - 1, m - 2] = jnp.zeros((C, W), bf16)

    wr = [jnp.concatenate([w_ref[r, s] for s in range(3)], axis=0).astype(f32) for r in range(3)]
    for a in range(n):
        ut[a] = _lin(g[a], wr).T.astype(bf16)

    lane = jax.lax.broadcasted_iota(jnp.int32, (8, 128), 1)

    def tf_pieces(t, vref):
        sp = (t + NS - 1) % NS
        sc = t % NS
        pieces = []
        for cc in range(nc):
            def piece(cc=cc):
                rs = pl.ds(cc * 16, 16)
                prev_p = prev_m = None
                for j in range(nj):
                    ls = pl.ds(j * 128, 128)
                    d = [xbuf[sp, m - 2 + i, rs, ls] for i in range(2)]
                    d += [xbuf[sc, i, rs, ls] for i in range(m)]
                    d = [v.astype(f32) for v in d]
                    vs = [v.astype(bf16) for v in _in_tf(bt, d)]
                    cur_p, cur_m = [], []
                    for a in range(n):
                        vref[a, pl.ds(C + cc * 16, 16), ls] = vs[a]
                        u = pltpu.bitcast(vs[a], jnp.uint32)
                        rp = pltpu.roll(u, 1, 1)
                        rm = pltpu.roll(u, 127, 1)
                        left = jnp.zeros_like(rp) if j == 0 else prev_p[a]
                        vref[a, rs, ls] = pltpu.bitcast(jnp.where(lane == 0, left, rp), bf16)
                        if j > 0:
                            vref[a, pl.ds(2 * C + cc * 16, 16), pl.ds((j - 1) * 128, 128)] = (
                                pltpu.bitcast(jnp.where(lane == 127, rm, prev_m[a]), bf16))
                        if j == nj - 1:
                            vref[a, pl.ds(2 * C + cc * 16, 16), ls] = pltpu.bitcast(
                                jnp.where(lane == 127, jnp.zeros_like(rm), rm), bf16)
                        cur_p.append(rp)
                        cur_m.append(rm)
                    prev_p, prev_m = cur_p, cur_m
            pieces.append(piece)
        return pieces

    def inv_pieces(mref, oref):
        pieces = []
        for cc in range(nc):
            def piece(cc=cc):
                rs = pl.ds(cc * 16, 16)
                for j in range(nj):
                    ls = pl.ds(j * 128, 128)
                    ys = _out_tf(at, [mref[a, rs, ls] for a in range(n)])
                    for i in range(m):
                        oref[i, rs, ls] = ys[i].astype(bf16)
            pieces.append(piece)
        return pieces

    def step(t, p, do_tf, do_mm, do_inv):
        tfp = tf_pieces(t + 1, vb[1 - p]) if do_tf else []
        ivp = inv_pieces(mb[1 - p], ob[1 - p]) if do_inv else []
        for a in range(n):
            if do_mm:
                mb[p][a] = jnp.dot(ut[a], vb[p][a], preferred_element_type=f32)
            for q in range(a * nc // n, (a + 1) * nc // n):
                if tfp:
                    tfp[q]()
                if ivp:
                    ivp[q]()

    first.wait()
    in_wait(0)
    step(-1, 1, True, False, False)
    in_wait(1)
    if nt > 3:
        in_start(3)
    step(0, 0, True, True, False)

    def dyn_start(c):
        @pl.when(c < nt - 1)
        def _():
            in_copy(c, m).start()

        @pl.when(c == nt - 1)
        def _():
            in_start(nt - 1)

    def dyn_wait(c):
        @pl.when(c < nt - 1)
        def _():
            in_copy(c, m).wait()

        if nin_last > 0:
            @pl.when(c == nt - 1)
            def _():
                in_copy(nt - 1, nin_last).wait()

    def body(k, carry):
        for p in (1, 0):
            t = 2 * k + 2 - p
            dyn_wait(t + 1)
            dyn_start(t + 3)

            @pl.when(t >= 3)
            def _():
                out_copy(t - 3, 1 - p, m).wait()

            step(t, p, True, True, True)
            out_copy(t - 1, 1 - p, m).start()
        return carry

    assert nt % 2 == 0 and nt >= 4
    jax.lax.fori_loop(0, (nt - 2) // 2, body, 0)
    t = nt - 1
    out_copy(t - 3, 0, m).wait()
    step(t, 1, False, True, True)
    out_copy(t - 1, 0, m).start()
    out_copy(t - 2, 1, m).wait()
    step(t + 1, 0, False, False, True)
    out_copy(t, 1, nout_last).start()
    out_copy(t - 1, 0, m).wait()
    out_copy(t, 1, nout_last).wait()


@jax.jit
def pallas_standalone__winograd__vision_kernel(x: jax.Array, w: jax.Array):
    N, H, W, C = x.shape
    K = w.shape[-1]
    assert N == 1 and K == C
    m = M_TILE
    n = m + 2
    xt = x.reshape(H, W, C).transpose(0, 2, 1)
    bf16, f32 = jnp.bfloat16, jnp.float32
    out = pl.pallas_call(
        functools.partial(_kernel, H=H, C=C, W=W, m=m),
        out_shape=jax.ShapeDtypeStruct((H, K, W), x.dtype),
        in_specs=[pl.BlockSpec(memory_space=pl.ANY),
                  pl.BlockSpec(memory_space=pltpu.VMEM)],
        out_specs=pl.BlockSpec(memory_space=pl.ANY),
        scratch_shapes=[
            pltpu.VMEM((4, m, C, W), bf16),
            pltpu.VMEM((n, K, 3 * C), bf16),
            pltpu.VMEM((n, 3 * C, W), bf16),
            pltpu.VMEM((n, 3 * C, W), bf16),
            pltpu.VMEM((n, K, W), f32),
            pltpu.VMEM((n, K, W), f32),
            pltpu.VMEM((m, K, W), bf16),
            pltpu.VMEM((m, K, W), bf16),
            pltpu.SemaphoreType.DMA((4,)),
            pltpu.SemaphoreType.DMA((2,)),
        ],
        compiler_params=pltpu.CompilerParams(vmem_limit_bytes=100 * 2**20),
    )(xt, w)
    return out.transpose(0, 2, 1).reshape(N, H, W, K)
```

```python
import functools
from fractions import Fraction

import numpy as np
import jax
import jax.numpy as jnp
import jax.experimental.pallas as pl
import jax.experimental.pallas.tpu as pltpu


M_TILE = 6
_PTS = {2: [0, 1, -1], 4: [0, 1, -1, 2, -2],
        6: [0, 1, -1, 2, -2, Fraction(1, 2), Fraction(-1, 2)]}


def _polymul(a, b):
    out = [Fraction(0)] * (len(a) + len(b) - 1)
    for i, x in enumerate(a):
        for j, y in enumerate(b):
            out[i + j] += x * y
    return out


def _wino(m, pts):
    n = m + 2
    pts = [Fraction(p) for p in pts]
    at = [[pts[j] ** i if j < n - 1 else Fraction(int(i == m - 1))
           for j in range(n)] for i in range(m)]
    g, bt = [], []
    for i in range(n - 1):
        den = Fraction(1)
        q = [Fraction(1)]
        for k in range(n - 1):
            if k != i:
                den *= pts[i] - pts[k]
                q = _polymul(q, [-pts[k], Fraction(1)])
        g.append([pts[i] ** j / den for j in range(3)])
        bt.append(q + [Fraction(0)] * (n - len(q)))
    g.append([Fraction(0), Fraction(0), Fraction(1)])
    q = [Fraction(1)]
    for p in pts:
        q = _polymul(q, [-p, Fraction(1)])
    bt.append(q)
    return at, g, bt


def _lin(coefs, vals):
    acc = None
    terms = sorted([(c, v) for c, v in zip(coefs, vals) if c != 0],
                   key=lambda t: 0 if t[0] == 1 else 1)
    for c, v in terms:
        if acc is None:
            acc = v if c == 1 else v * float(c)
        elif c == 1:
            acc = acc + v
        elif c == -1:
            acc = acc - v
        else:
            acc = acc + v * float(c)
    return acc


def _in_tf(bt, d):
    n = len(d)
    out = [None] * n
    out[0] = _lin(bt[0], d)
    out[n - 1] = _lin(bt[n - 1], d)
    for a in range(1, n - 1, 2):
        ev = [c if j % 2 == 0 else 0 for j, c in enumerate(bt[a])]
        od = [c if j % 2 == 1 else 0 for j, c in enumerate(bt[a])]
        assert all(bt[a + 1][j] == (-od[j] if j % 2 else ev[j]) for j in range(n)) or \
            all(bt[a + 1][j] == (od[j] if j % 2 else -ev[j]) for j in range(n))
        e, o = _lin(ev, d), _lin(od, d)
        out[a] = e + o
        if all(bt[a + 1][j] == (-od[j] if j % 2 else ev[j]) for j in range(n)):
            out[a + 1] = e - o
        else:
            out[a + 1] = o - e
    return out


def _out_tf(at, mm):
    n = len(mm)
    s = [mm[a] + mm[a + 1] for a in range(1, n - 1, 2)]
    df = [mm[a] - mm[a + 1] for a in range(1, n - 1, 2)]
    ys = []
    for i, row in enumerate(at):
        src = s if i % 2 == 0 else df
        coefs = [row[a] for a in range(1, n - 1, 2)] + [row[0], row[n - 1]]
        ys.append(_lin(coefs, src + [mm[0], mm[n - 1]]))
    return ys


def _kernel(x_hbm, w_ref, o_hbm, xbuf, ut, v0, v1, m0, m1, ob0, ob1, isem, osem,
            *, H, C, W, m):
    n = m + 2
    at, g, bt = _wino(m, _PTS[m])
    nt = -(-H // m)
    nin_last = H - (m * (nt - 1) + 1)
    nout_last = H - m * (nt - 1)
    NS = 4
    nj = W // 128
    nc = C // 16
    vb, mb, ob = (v0, v1), (m0, m1), (ob0, ob1)
    f32, bf16 = jnp.float32, jnp.bfloat16

    def in_copy(c, rows):
        slot = c % NS
        return pltpu.make_async_copy(
            x_hbm.at[pl.ds(m * c + 1, rows)], xbuf.at[slot, pl.ds(0, rows)], isem.at[slot])

    def in_start(c):
        if c < nt - 1:
            in_copy(c, m).start()
        elif c == nt - 1:
            if nin_last > 0:
                in_copy(c, nin_last).start()
            xbuf[c % NS, nin_last:] = jnp.zeros((m - nin_last, C, W), bf16)

    def in_wait(c):
        if c < nt - 1:
            in_copy(c, m).wait()
        elif c == nt - 1 and nin_last > 0:
            in_copy(c, nin_last).wait()

    def out_copy(t, p, rows):
        return pltpu.make_async_copy(
            ob[p].at[pl.ds(0, rows)], o_hbm.at[pl.ds(m * t, rows)], osem.at[p])

    first = pltpu.make_async_copy(
        x_hbm.at[pl.ds(0, 1)], xbuf.at[NS - 1, pl.ds(m - 1, 1)], isem.at[NS - 1])
    first.start()
    for c in range(3):
        in_start(c)
    xbuf[NS - 1, m - 2] = jnp.zeros((C, W), bf16)

    ri = jax.lax.broadcasted_iota(jnp.int32, (C, C), 0)
    ci = jax.lax.broadcasted_iota(jnp.int32, (C, C), 1)
    src = (ri & ~15) + ((ri & 1) << 3) + ((ri & 15) >> 1)
    perm = jnp.where(ci == src, 1.0, 0.0).astype(bf16)
    wr = [jnp.concatenate([jnp.dot(perm, w_ref[r, s], preferred_element_type=f32)
                           for s in range(3)], axis=0) for r in range(3)]
    for a in range(n):
        ut[a] = pltpu.bitcast(_lin(g[a], wr).T.astype(bf16), jnp.uint32)

    lane = jax.lax.broadcasted_iota(jnp.int32, (8, 128), 1)
    C2 = C // 2

    def tf_pieces(t, vref):
        sp = (t + NS - 1) % NS
        sc = t % NS
        pieces = []
        for cc in range(nc):
            def piece(cc=cc):
                rs = pl.ds(cc * 8, 8)
                prev_p = prev_m = None
                for jj in range(nj // 2):
                    ls = pl.ds(jj * 256, 256)
                    vh = []
                    for hf in range(2):
                        cs = pl.ds(cc * 16 + hf * 8, 8)
                        d = [xbuf[sp, m - 2 + i, cs, ls] for i in range(2)]
                        d += [xbuf[sc, i, cs, ls] for i in range(m)]
                        vh.append(_in_tf(bt, [v.astype(f32) for v in d]))
                    vs = [pltpu.pack_elementwise([vh[0][a], vh[1][a]], packed_dtype=bf16)
                          for a in range(n)]
                    for j in (2 * jj, 2 * jj + 1):
                        ls = pl.ds(j * 128, 128)
                        cur_p, cur_m = [], []
                        for a in range(n):
                            u = vs[a][:, (j % 2) * 128:(j % 2 + 1) * 128]
                            vref[a, pl.ds(C2 + cc * 8, 8), ls] = u
                            rp = pltpu.roll(u, 1, 1)
                            rm = pltpu.roll(u, 127, 1)
                            left = jnp.zeros_like(rp) if j == 0 else prev_p[a]
                            vref[a, rs, ls] = jnp.where(lane == 0, left, rp)
                            if j > 0:
                                vref[a, pl.ds(2 * C2 + cc * 8, 8), pl.ds((j - 1) * 128, 128)] = (
                                    jnp.where(lane == 127, rm, prev_m[a]))
                            if j == nj - 1:
                                vref[a, pl.ds(2 * C2 + cc * 8, 8), ls] = (
                                    jnp.where(lane == 127, jnp.zeros_like(rm), rm))
                            cur_p.append(rp)
                            cur_m.append(rm)
                        prev_p, prev_m = cur_p, cur_m
            pieces.append(piece)
        return pieces

    def inv_pieces(mref, oref):
        pieces = []
        for cc in range(nc):
            def piece(cc=cc):
                for hf in range(2):
                    rs = pl.ds(cc * 16 + hf * 8, 8)
                    for jj in range(nj // 2):
                        ls = pl.ds(jj * 256, 256)
                        ys = _out_tf(at, [mref[a, rs, ls] for a in range(n)])
                        for i in range(m):
                            oref[i, rs, ls] = ys[i].astype(bf16)
            pieces.append(piece)
        return pieces

    def step(t, p, do_tf, do_mm, do_inv):
        tfp = tf_pieces(t + 1, vb[1 - p]) if do_tf else []
        ivp = inv_pieces(mb[1 - p], ob[1 - p]) if do_inv else []
        for a in range(n):
            if do_mm:
                mb[p][a] = jnp.dot(pltpu.bitcast(ut[a], bf16), pltpu.bitcast(vb[p][a], bf16),
                                   preferred_element_type=f32)
            for q in range(a * nc // n, (a + 1) * nc // n):
                if tfp:
                    tfp[q]()
                if ivp:
                    ivp[q]()

    first.wait()
    in_wait(0)
    step(-1, 1, True, False, False)
    in_wait(1)
    if nt > 3:
        in_start(3)
    step(0, 0, True, True, False)

    def dyn_start(c):
        @pl.when(c < nt - 1)
        def _():
            in_copy(c, m).start()

        @pl.when(c == nt - 1)
        def _():
            in_start(nt - 1)

    def dyn_wait(c):
        @pl.when(c < nt - 1)
        def _():
            in_copy(c, m).wait()

        if nin_last > 0:
            @pl.when(c == nt - 1)
            def _():
                in_copy(nt - 1, nin_last).wait()

    def body(k, carry):
        for p in (1, 0):
            t = 2 * k + 2 - p
            dyn_wait(t + 1)
            dyn_start(t + 3)

            @pl.when(t >= 3)
            def _():
                out_copy(t - 3, 1 - p, m).wait()

            step(t, p, True, True, True)
            out_copy(t - 1, 1 - p, m).start()
        return carry

    assert nt % 2 == 0 and nt >= 4
    jax.lax.fori_loop(0, (nt - 2) // 2, body, 0)
    t = nt - 1
    out_copy(t - 3, 0, m).wait()
    step(t, 1, False, True, True)
    out_copy(t - 1, 0, m).start()
    out_copy(t - 2, 1, m).wait()
    step(t + 1, 0, False, False, True)
    out_copy(t, 1, nout_last).start()
    out_copy(t - 1, 0, m).wait()
    out_copy(t, 1, nout_last).wait()


@jax.jit
def pallas_standalone__winograd__vision_kernel(x: jax.Array, w: jax.Array):
    N, H, W, C = x.shape
    K = w.shape[-1]
    assert N == 1 and K == C
    m = M_TILE
    n = m + 2
    xt = x.reshape(H, W, C).transpose(0, 2, 1)
    bf16, f32 = jnp.bfloat16, jnp.float32
    out = pl.pallas_call(
        functools.partial(_kernel, H=H, C=C, W=W, m=m),
        out_shape=jax.ShapeDtypeStruct((H, K, W), x.dtype),
        in_specs=[pl.BlockSpec(memory_space=pl.ANY),
                  pl.BlockSpec(memory_space=pltpu.VMEM)],
        out_specs=pl.BlockSpec(memory_space=pl.ANY),
        scratch_shapes=[
            pltpu.VMEM((4, m, C, W), bf16),
            pltpu.VMEM((n, K // 2, 3 * C), jnp.uint32),
            pltpu.VMEM((n, 3 * C // 2, W), jnp.uint32),
            pltpu.VMEM((n, 3 * C // 2, W), jnp.uint32),
            pltpu.VMEM((n, K, W), f32),
            pltpu.VMEM((n, K, W), f32),
            pltpu.VMEM((m, K, W), bf16),
            pltpu.VMEM((m, K, W), bf16),
            pltpu.SemaphoreType.DMA((4,)),
            pltpu.SemaphoreType.DMA((2,)),
        ],
        compiler_params=pltpu.CompilerParams(vmem_limit_bytes=100 * 2**20),
    )(xt, w)
    return out.transpose(0, 2, 1).reshape(N, H, W, K)
```
